```python
import jax
import jax.numpy as jnp

def _softmax(x, axis=-1):
    return jax.nn.softmax(x, axis=axis)

def _gelu(x):
    return jax.nn.gelu(x, approximate=True)

def _silu(x):
    return jax.nn.silu(x)

def _sigmoid(x):
    return jax.nn.sigmoid(x)

def _layernorm(x, axis=-1, eps=1e-05):
    m = jnp.mean(x, axis=axis, keepdims=True)
    v = jnp.var(x, axis=axis, keepdims=True)
    return (x - m) / jnp.sqrt(v + eps)

def _scatter_add(tgt, idx, src, axis=0):
    return tgt.at[idx].add(src)

def _segment_sum(src, seg, n):
    return jax.ops.segment_sum(src, seg, n)

class _Rng:

    def __init__(self, key):
        self._k = key

    def _next(self):
        self._k, sub = jax.random.split(self._k)
        return sub

    def normal(self, shape):
        return jax.random.normal(self._next(), shape, dtype=jnp.bfloat16)

    def randint(self, lo, hi, shape):
        return jax.random.randint(self._next(), shape, lo, hi, dtype=jnp.int32)

    def uniform(self, shape, lo=0.0, hi=1.0):
        return jax.random.uniform(self._next(), shape, jnp.bfloat16, lo, hi)

    def permutation(self, n):
        return jax.random.permutation(self._next(), n)
kernel_name = 'standalone__dilated_atrous__vision'

def setup_inputs():
    _rng = _Rng(jax.random.key(int.from_bytes(__import__("os").urandom(4), "little")))
    _w = lambda a: (lambda t: t.astype(jnp.bfloat16) if jnp.issubdtype(t.dtype, jnp.floating) else t)(jnp.asarray(a))
    H = W = 384
    C = 384
    k = 1
    return {'x': _w((lambda *s: _rng.normal(s) * 0.05)(1, H, W, C)), 'w': _w((lambda *s: _rng.normal(s) * 0.05)(k, k, C, C) * (1.0 / (k * C ** 0.5)))}

def reference(x, w):
    B, H, W, C = x.shape
    k = 1
    rate = 2
    pad = (k - 1) * rate // 2
    xp = jnp.pad(x, ((0, 0), (pad, pad), (pad, pad), (0, 0)))
    out = jnp.zeros_like(x)
    for i in range(k):
        for j in range(k):
            tap = xp[:, i * rate:i * rate + H, j * rate:j * rate + W, :].copy()
            out = out + jnp.einsum('bhwc,co->bhwo', tap, w[i, j])
    return out
```

```python
import jax
import jax.numpy as jnp
import jax.experimental.pallas as pl
import jax.experimental.pallas.tpu as pltpu


def _conv1x1_kernel(x_ref, w_ref, o_ref):
    o_ref[...] = jnp.dot(
        x_ref[...], w_ref[...], preferred_element_type=jnp.float32
    ).astype(o_ref.dtype)


@jax.jit
def pallas_standalone__dilated_atrous__vision_kernel(
    x: jax.Array,
    w: jax.Array,
):
    B, H, W, C = x.shape
    O = w.shape[-1]
    M = B * H * W
    TM = 2048
    x2 = x.reshape(M, C)
    w2 = w.reshape(C, O)
    out = pl.pallas_call(
        _conv1x1_kernel,
        grid=(M // TM,),
        in_specs=[
            pl.BlockSpec((TM, C), lambda i: (i, 0)),
            pl.BlockSpec((C, O), lambda i: (0, 0)),
        ],
        out_specs=pl.BlockSpec((TM, O), lambda i: (i, 0)),
        out_shape=jax.ShapeDtypeStruct((M, O), x.dtype),
        compiler_params=pltpu.CompilerParams(
            dimension_semantics=("arbitrary",),
            vmem_limit_bytes=64 * 1024 * 1024,
        ),
    )(x2, w2)
    return out.reshape(B, H, W, O)
```

```python
import jax
import jax.numpy as jnp
from jax import lax
import jax.experimental.pallas as pl
import jax.experimental.pallas.tpu as pltpu

GROUP_ROWS = 4096
CHUNK_ROWS = 128
WRITE_ROWS = 32
SUB_STEPS = 4


def _conv1x1_kernel(x_hbm, w_hbm, o_hbm, buf, wbuf, rsem, wsem, osem):
    n_chunks, n_groups, chunk_rows, c = buf.shape
    writes_per_chunk = chunk_rows // WRITE_ROWS
    groups_per_sub = n_groups // SUB_STEPS
    switch = n_chunks // 2

    def read(r):
        start = pl.multiple_of(r * chunk_rows, chunk_rows)
        return pltpu.make_async_copy(
            x_hbm.at[:, pl.ds(start, chunk_rows)], buf.at[r], rsem.at[r]
        )

    def write(r, j):
        start = pl.multiple_of(r * chunk_rows + j * WRITE_ROWS, WRITE_ROWS)
        return pltpu.make_async_copy(
            buf.at[r, :, pl.ds(j * WRITE_ROWS, WRITE_ROWS)],
            o_hbm.at[:, pl.ds(start, WRITE_ROWS)],
            osem.at[0],
        )

    def start_writes(r, carry):
        for j in range(writes_per_chunk):
            write(r, j).start()
        return carry

    def wait_writes(r, carry):
        for j in range(writes_per_chunk):
            write(r, j).wait()
        return carry

    def start_read(r, carry):
        read(r).start()
        return carry

    load_w = pltpu.make_async_copy(w_hbm, wbuf, wsem.at[0])
    load_w.start()
    lax.fori_loop(0, n_chunks, start_read, None)
    load_w.wait()

    def step(r, carry):
        @pl.when(r == switch)
        def _():
            read(n_chunks - 1).wait()
            lax.fori_loop(0, switch, start_writes, None)

        @pl.when(r < n_chunks - 1)
        def _():
            read(r).wait()

        for s in range(SUB_STEPS):
            groups = pl.ds(s * groups_per_sub, groups_per_sub)
            a = buf[r, groups].reshape(groups_per_sub * chunk_rows, c)
            y = jnp.dot(a, wbuf[...], preferred_element_type=jnp.float32)
            buf[r, groups] = y.astype(buf.dtype).reshape(groups_per_sub, chunk_rows, c)

        @pl.when(r >= switch)
        def _():
            start_writes(r, None)

        return carry

    lax.fori_loop(0, n_chunks, step, None)
    lax.fori_loop(0, n_chunks, wait_writes, None)


@jax.jit
def pallas_standalone__dilated_atrous__vision_kernel(
    x: jax.Array,
    w: jax.Array,
):
    B, H, W, C = x.shape
    assert w.shape == (1, 1, C, C)
    n_groups = (B * H * W) // GROUP_ROWS
    assert n_groups * GROUP_ROWS == B * H * W and n_groups % SUB_STEPS == 0
    n_chunks = GROUP_ROWS // CHUNK_ROWS

    out = pl.pallas_call(
        _conv1x1_kernel,
        in_specs=[
            pl.BlockSpec(memory_space=pl.ANY),
            pl.BlockSpec(memory_space=pl.ANY),
        ],
        out_specs=pl.BlockSpec(memory_space=pl.ANY),
        out_shape=jax.ShapeDtypeStruct((n_groups, GROUP_ROWS, C), x.dtype),
        scratch_shapes=[
            pltpu.VMEM((n_chunks, n_groups, CHUNK_ROWS, C), x.dtype),
            pltpu.VMEM((C, C), w.dtype),
            pltpu.SemaphoreType.DMA((n_chunks,)),
            pltpu.SemaphoreType.DMA((1,)),
            pltpu.SemaphoreType.DMA((1,)),
        ],
        compiler_params=pltpu.CompilerParams(vmem_limit_bytes=120 * 1024 * 1024),
    )(x.reshape(n_groups, GROUP_ROWS, C), w.reshape(C, C))
    return out.reshape(B, H, W, C)
```

```python
import jax
import jax.numpy as jnp
from jax import lax
import jax.experimental.pallas as pl
import jax.experimental.pallas.tpu as pltpu

GROUPS = 6
RUN_ROWS = 48
STEP_RUNS = 8
EARLY_READS = 4
LEAD_WRITES = 32


def _conv1x1_kernel(x_hbm, w_hbm, o_hbm, buf, w_buf, early_sems, sems):
    groups, n_runs, run_rows, channels = buf.shape
    n_steps = n_runs // STEP_RUNS
    half_steps = n_steps // 2
    half_runs = half_steps * STEP_RUNS
    early_steps = half_steps // EARLY_READS
    early_runs = early_steps * STEP_RUNS

    def read(start, size, sem):
        runs = pl.ds(start, size)
        return pltpu.make_async_copy(x_hbm.at[:, runs], buf.at[:, runs], sem)

    def early_read(k):
        return read(k * early_runs, early_runs, early_sems.at[k])

    def write(j):
        return pltpu.make_async_copy(buf.at[:, j], o_hbm.at[:, j], sems.at[0])

    def matmul(step):
        runs = pl.ds(step * STEP_RUNS, STEP_RUNS)
        rows = buf[:, runs].reshape(groups * STEP_RUNS * run_rows, channels)
        out = jnp.dot(rows, w_buf[...], preferred_element_type=jnp.float32)
        buf[:, runs] = out.astype(buf.dtype).reshape(
            groups, STEP_RUNS, run_rows, channels
        )

    def loop(lo, hi, fn):
        lax.fori_loop(lo, hi, lambda i, _: fn(i), None)

    w_read = pltpu.make_async_copy(w_hbm, w_buf, sems.at[1])
    late_read = read(half_runs, n_runs - half_runs - 1, sems.at[2])
    last_read = read(n_runs - 1, 1, sems.at[3])
    w_read.start()
    loop(0, EARLY_READS, lambda k: early_read(k).start())
    late_read.start()
    last_read.start()
    w_read.wait()

    def early_piece(k):
        early_read(k).wait()
        loop(k * early_steps, (k + 1) * early_steps, matmul)

    loop(0, EARLY_READS, early_piece)

    late_read.wait()
    loop(0, LEAD_WRITES, lambda j: write(j).start())
    last_read.wait()

    def queued(step):
        return jnp.minimum(
            LEAD_WRITES + 2 * STEP_RUNS * (step - half_steps), step * STEP_RUNS
        )

    def late_step(step):
        matmul(step)
        loop(queued(step), queued(step + 1), lambda j: write(j).start())

    loop(half_steps, n_steps, late_step)
    loop(0, n_runs, lambda j: write(j).wait())


@jax.jit
def pallas_standalone__dilated_atrous__vision_kernel(
    x: jax.Array,
    w: jax.Array,
):
    B, H, W, C = x.shape
    assert w.shape == (1, 1, C, C)
    n_runs = B * H * W // (GROUPS * RUN_ROWS)
    assert GROUPS * n_runs * RUN_ROWS == B * H * W
    assert n_runs % (2 * EARLY_READS * STEP_RUNS) == 0
    assert LEAD_WRITES <= n_runs // 2
    view = (GROUPS, n_runs, RUN_ROWS, C)

    out = pl.pallas_call(
        _conv1x1_kernel,
        in_specs=[
            pl.BlockSpec(memory_space=pl.ANY),
            pl.BlockSpec(memory_space=pl.ANY),
        ],
        out_specs=pl.BlockSpec(memory_space=pl.ANY),
        out_shape=jax.ShapeDtypeStruct(view, x.dtype),
        scratch_shapes=[
            pltpu.VMEM(view, x.dtype),
            pltpu.VMEM((C, C), w.dtype),
            pltpu.SemaphoreType.DMA((EARLY_READS,)),
            pltpu.SemaphoreType.DMA((4,)),
        ],
        compiler_params=pltpu.CompilerParams(vmem_limit_bytes=120 * 1024 * 1024),
    )(x.reshape(view), w.reshape(C, C))
    return out.reshape(B, H, W, C)
```
